```python
import os as _os
_os.environ.setdefault('JAX_PLATFORMS', 'cpu')
import jax
import jax.numpy as jnp

def _softmax(x, axis=-1):
    return jax.nn.softmax(x, axis=axis)

def _gelu(x):
    return jax.nn.gelu(x, approximate=True)

def _silu(x):
    return jax.nn.silu(x)

def _sigmoid(x):
    return jax.nn.sigmoid(x)

def _layernorm(x, axis=-1, eps=1e-05):
    m = jnp.mean(x, axis=axis, keepdims=True)
    v = jnp.var(x, axis=axis, keepdims=True)
    return (x - m) / jnp.sqrt(v + eps)

def _scatter_add(tgt, idx, src, axis=0):
    return tgt.at[idx].add(src)

def _segment_sum(src, seg, n):
    return jax.ops.segment_sum(src, seg, n)

class _Rng:

    def __init__(self, key):
        self._k = key

    def _next(self):
        self._k, sub = jax.random.split(self._k)
        return sub

    def normal(self, shape):
        return jax.random.normal(self._next(), shape, dtype=jnp.bfloat16)

    def randint(self, lo, hi, shape):
        return jax.random.randint(self._next(), shape, lo, hi, dtype=jnp.int32)

    def uniform(self, shape, lo=0.0, hi=1.0):
        return jax.random.uniform(self._next(), shape, jnp.bfloat16, lo, hi)

    def permutation(self, n):
        return jax.random.permutation(self._next(), n)
kernel_name = 'concat_heads__ssm_conv_s5__memory_aug_recurrent_mem_tr__prompt'

def setup_inputs():
    _rng = _Rng(jax.random.key(int.from_bytes(__import__("os").urandom(4), "little")))
    _w = lambda a: (lambda t: t.astype(jnp.bfloat16) if jnp.issubdtype(t.dtype, jnp.floating) else t)(jnp.asarray(a))

    def _A_setup():
        B, S, D = (1, 2048, 1024)
        P = D
        Lambda_re = -0.5 * jnp.exp((lambda *s: _rng.normal(s) * 0.8)(P))
        Lambda_im = (lambda *s: _rng.normal(s) * 0.8)(P) * 1.0
        B_re = (lambda *s: _rng.normal(s) * 0.8)(P, D) * D ** (-0.5)
        B_im = (lambda *s: _rng.normal(s) * 0.8)(P, D) * D ** (-0.5)
        C_re = (lambda *s: _rng.normal(s) * 0.8)(D, P) * P ** (-0.5)
        C_im = (lambda *s: _rng.normal(s) * 0.8)(D, P) * P ** (-0.5)
        log_dt = (lambda *s: _rng.normal(s) * 0.8)(P) * 0.3 - 2.0
        Dskip = (lambda *s: _rng.normal(s) * 0.8)(D)
        return {'x': _w((lambda *s: _rng.normal(s) * 0.05)(B, S, D)), 'Lambda_re': _w(Lambda_re), 'Lambda_im': _w(Lambda_im), 'B_re': _w(B_re), 'B_im': _w(B_im), 'C_re': _w(C_re), 'C_im': _w(C_im), 'log_dt': _w(log_dt), 'Dskip': _w(Dskip)}
    _A_in = _A_setup()

    def _B_setup():
        B, S, Dm = (1, 2048, 1024)
        H, Dh = (32, 128)
        M, seg = (8, 32)
        seg = min(seg, S)
        S = S // seg * seg
        return {'x': _w((lambda *s: _rng.normal(s) * 0.05)(B, S, Dm)), 'mem0': _w((lambda *s: _rng.normal(s) * 0.8)(B, M, Dm)), 'Wq': _w((lambda *s: _rng.normal(s) * 1.6)(Dm, H, Dh) * Dm ** (-0.5)), 'Wk': _w((lambda *s: _rng.normal(s) * 1.6)(Dm, H, Dh) * Dm ** (-0.5)), 'Wv': _w((lambda *s: _rng.normal(s) * 0.8)(Dm, H, Dh) * Dm ** (-0.5)), 'Wo': _w((lambda *s: _rng.normal(s) * 0.8)(H, Dh, Dm) * (H * Dh) ** (-0.5)), 'seg_len': seg}
    _B_in = _B_setup()
    return {'A_x': _A_in['x'], 'A_Lambda_re': _A_in['Lambda_re'], 'A_Lambda_im': _A_in['Lambda_im'], 'A_B_re': _A_in['B_re'], 'A_B_im': _A_in['B_im'], 'A_C_re': _A_in['C_re'], 'A_C_im': _A_in['C_im'], 'A_log_dt': _A_in['log_dt'], 'A_Dskip': _A_in['Dskip'], 'B_x': _B_in['x'], 'B_mem0': _B_in['mem0'], 'B_Wq': _B_in['Wq'], 'B_Wk': _B_in['Wk'], 'B_Wv': _B_in['Wv'], 'B_Wo': _B_in['Wo'], 'B_seg_len': _B_in['seg_len']}

def reference(A_x, A_Lambda_re, A_Lambda_im, A_B_re, A_B_im, A_C_re, A_C_im, A_log_dt, A_Dskip, B_x, B_mem0, B_Wq, B_Wk, B_Wv, B_Wo, B_seg_len):

    def _A_ref(x, Lambda_re, Lambda_im, B_re, B_im, C_re, C_im, log_dt, Dskip):
        Bsz, L, H = x.shape
        Lam = Lambda_re + 1j * Lambda_im
        Bmat = B_re + 1j * B_im
        Cmat = C_re + 1j * C_im
        dt = jnp.exp(log_dt)
        Lam_bar = jnp.exp(dt * Lam)
        B_bar = ((Lam_bar - 1.0) / Lam)[:, None] * Bmat
        Bu = jnp.einsum('bld,pd->blp', x + 0j, B_bar)
        h = jnp.zeros_like(Bu[:, 0, :])
        hs = []
        for t in range(L):
            h = Lam_bar[None, :] * h + Bu[:, t, :]
            hs.append(h)
        hseq = jnp.stack(hs, 1)
        y = 2.0 * jnp.einsum('blp,dp->bld', hseq, Cmat).real + x * Dskip[None, None, :]
        return y

    def _B_ref(x, mem0, Wq, Wk, Wv, Wo, seg_len):
        B, S, Dm = x.shape
        H, Dh = (Wq.shape[1], Wq.shape[2])
        M = mem0.shape[1]
        scale = Dh ** (-0.5)
        n_seg = S // seg_len
        L = M + seg_len
        idx = jnp.arange(L)
        mask = (idx[:, None] < M) | (idx[:, None] >= idx[None, :])
        mem = mem0
        outs = []
        for s in range(n_seg):
            xs = x[:, s * seg_len:(s + 1) * seg_len, :].copy()
            h = jnp.concatenate([mem, xs], axis=1)
            q = jnp.einsum('btd,dhe->bhte', h, Wq)
            k = jnp.einsum('btd,dhe->bhte', h, Wk)
            v = jnp.einsum('btd,dhe->bhte', h, Wv)
            scores = jnp.einsum('bhqe,bhke->bhqk', q, k) * scale
            scores = jnp.where(mask[None, None], scores, -1000000000.0)
            p = _softmax(scores, axis=-1)
            o = jnp.einsum('bhqk,bhke->bhqe', p, v)
            o = jnp.einsum('bhte,hed->btd', o, Wo)
            mem = o[:, :M, :].copy()
            outs.append(o[:, M:, :])
        return jnp.concatenate(outs, axis=1)
    a = _A_ref(A_x, A_Lambda_re, A_Lambda_im, A_B_re, A_B_im, A_C_re, A_C_im, A_log_dt, A_Dskip)
    b = _B_ref(B_x, B_mem0, B_Wq, B_Wk, B_Wv, B_Wo, B_seg_len)
    return jnp.concatenate([a, b], axis=-1)
```

```python
import functools

import jax
import jax.numpy as jnp
import numpy as np
from jax import lax
import jax.experimental.pallas as pl
import jax.experimental.pallas.tpu as pltpu

F32 = jnp.float32
BF16 = jnp.bfloat16
U32 = jnp.uint32
HI16 = np.uint32(0xFFFF0000)
LO16 = np.uint32(0x0000FFFF)
NT = (((1,), (1,)), ((), ()))
NN = (((1,), (0,)), ((), ()))

NC = 8
TB = 32


def _dot(a, b, dims=NN):
    return lax.dot_general(a, b, dims, preferred_element_type=F32)


def _cmul(ar, ai, br, bi):
    return ar * br - ai * bi, ar * bi + ai * br


def _kernel(xa_hbm, lre_ref, lim_ref, bre_hbm, bim_hbm, cre_hbm, cim_hbm, ldt_ref, dsk_ref,
            xb_hbm, mem0_ref, wq_hbm, wk_hbm, wv_hbm, wo_hbm, out_hbm,
            xa, bw, cw, hloc, ya, par, xb, wqkv, wo, yb, hbuf, obuf,
            s_xa, s_bc, s_w, s_misc, s_out, *, S, D, H, M, SEG):
    LC = S // NC
    NB = LC // TB
    NSEG = S // SEG
    L = M + SEG
    HP = H // 2

    xa_src = xa_hbm.bitcast(U32)

    def xa_copy(b, c):
        sl = pl.ds(b * (TB // 2), TB // 2)
        return pltpu.make_async_copy(xa_src.at[c, sl, :], xa.at[sl, c, :], s_xa.at[b])

    bc_copies = [
        pltpu.make_async_copy(bre_hbm.bitcast(U32), bw.at[0], s_bc.at[0]),
        pltpu.make_async_copy(bim_hbm.bitcast(U32), bw.at[1], s_bc.at[1]),
        pltpu.make_async_copy(cre_hbm.bitcast(U32), cw.at[0], s_bc.at[2]),
        pltpu.make_async_copy(cim_hbm.bitcast(U32), cw.at[1], s_bc.at[3]),
    ]
    w_copies = []
    for i, w in enumerate((wq_hbm, wk_hbm, wv_hbm)):
        src = w.bitcast(U32)
        w_copies.append([pltpu.make_async_copy(src.at[:, r, :], wqkv.at[i, r], s_w.at[i])
                         for r in range(H)])
    wo_copy = pltpu.make_async_copy(wo_hbm.bitcast(U32), wo, s_misc.at[0])
    xb_copy = pltpu.make_async_copy(xb_hbm, xb, s_misc.at[1])

    for c in range(NC):
        xa_copy(0, c).start()
    bc_copies[0].start()
    bc_copies[1].start()
    for b in range(1, NB):
        for c in range(NC):
            xa_copy(b, c).start()
    bc_copies[2].start()
    bc_copies[3].start()
    for cs in w_copies:
        for cp in cs:
            cp.start()
    wo_copy.start()
    xb_copy.start()

    lre = lre_ref[...].astype(F32)
    lim = lim_ref[...].astype(F32)
    dt = jnp.exp(ldt_ref[...].astype(F32)).astype(BF16).astype(F32)
    mag = jnp.exp(dt * lre)
    ar = mag * jnp.cos(dt * lim)
    ai = mag * jnp.sin(dt * lim)
    den = lre * lre + lim * lim
    nr = ar - 1.0
    gr = 2.0 * (nr * lre + ai * lim) / den
    gi = 2.0 * (ai * lre - nr * lim) / den
    for i, v in enumerate((ar, ai, gr, gi)):
        par[i] = jnp.broadcast_to(v, (NC, D))
    par[4] = jnp.broadcast_to(dsk_ref[...].astype(F32), (NC, D))

    def x_block(b):
        w = xa[pl.ds(b * (TB // 2), TB // 2)]
        ev = pltpu.bitcast(w << 16, F32)
        od = pltpu.bitcast(w & HI16, F32)
        return jnp.stack([ev, od], axis=1).reshape(TB, NC, D)

    bc_copies[0].wait()
    bc_copies[1].wait()
    par[5] = jnp.zeros((NC, D), F32)
    par[6] = jnp.zeros((NC, D), F32)

    def a1(b, _):
        for c in range(NC):
            xa_copy(b, c).wait()
        x = x_block(b).reshape(TB * NC, D).astype(BF16)
        for j in range(D // 128):
            ls = pl.ds(j * 128, 128)
            ur = _dot(x, pltpu.bitcast(bw[0, pl.ds(j * 64, 64), :], BF16), NT).reshape(TB, NC, 128)
            ui = _dot(x, pltpu.bitcast(bw[1, pl.ds(j * 64, 64), :], BF16), NT).reshape(TB, NC, 128)
            lr, li = par[0, :, ls], par[1, :, ls]
            hr, hi = par[5, :, ls], par[6, :, ls]
            for t in range(TB):
                hr, hi = lr * hr - li * hi + ur[t], lr * hi + li * hr + ui[t]
                hloc[0, b * TB + t, :, ls] = hr
                hloc[1, b * TB + t, :, ls] = hi
            par[5, :, ls] = hr
            par[6, :, ls] = hi

    lax.fori_loop(0, NB, a1, None)

    pr, pi = par[0], par[1]
    n = 1
    while n < LC:
        pr, pi = pr * pr - pi * pi, 2.0 * pr * pi
        n *= 2
    sub = lax.broadcasted_iota(jnp.int32, (NC, D), 0)
    er = jnp.where(sub >= 1, pltpu.roll(par[5], 1, 0), 0.0)
    ei = jnp.where(sub >= 1, pltpu.roll(par[6], 1, 0), 0.0)
    d = 1
    while d < NC:
        sr = jnp.where(sub >= d, pltpu.roll(er, d, 0), 0.0)
        si = jnp.where(sub >= d, pltpu.roll(ei, d, 0), 0.0)
        mr, mi = _cmul(pr, pi, sr, si)
        er, ei = er + mr, ei + mi
        pr, pi = pr * pr - pi * pi, 2.0 * pr * pi
        d *= 2
    par[5] = er
    par[6] = ei

    bc_copies[2].wait()
    bc_copies[3].wait()
    for cs in w_copies:
        for cp in cs:
            cp.wait()

    def ya_copy(b, c):
        sl = pl.ds(b * TB, TB)
        return pltpu.make_async_copy(ya.at[sl, c, :], out_hbm.at[c, sl, pl.ds(0, D)], s_out.at[0])

    def a2(b, _):
        lr, li, g_r, g_i = par[0], par[1], par[2], par[3]
        cr, ci = par[5], par[6]
        zr, zi = [], []
        for t in range(TB):
            cr, ci = _cmul(lr, li, cr, ci)
            hr = hloc[0, b * TB + t] + cr
            hi = hloc[1, b * TB + t] + ci
            zr.append(g_r * hr - g_i * hi)
            zi.append(g_r * hi + g_i * hr)
        par[5] = cr
        par[6] = ci
        zr = jnp.concatenate(zr, axis=0).astype(BF16)
        zi = jnp.concatenate(zi, axis=0).astype(BF16)
        y = _dot(zr, pltpu.bitcast(cw[0], BF16), NT) - _dot(zi, pltpu.bitcast(cw[1], BF16), NT)
        skip = (x_block(b) * par[4][None]).astype(BF16).astype(F32)
        ya[pl.ds(b * TB, TB)] = y.reshape(TB, NC, D) + skip
        for c in range(NC):
            ya_copy(b, c).start()
        for i in range(3):
            for r in range(HP // NB):
                p = b * (HP // NB) + r
                e = wqkv[i, p]
                o = wqkv[i, HP + p]
                wqkv[i, p] = (e & LO16) | (o << 16)
                wqkv[i, HP + p] = (e >> 16) | (o & HI16)

    lax.fori_loop(0, NB, a2, None)

    wo_copy.wait()
    xb_copy.wait()
    hbuf[pl.ds(0, M), :] = mem0_ref[...].astype(F32)
    scale = 128.0 ** -0.5

    def yb_copy(s):
        per = LC // SEG
        return pltpu.make_async_copy(
            yb.at[pl.ds(s * SEG, SEG), :],
            out_hbm.at[s // per, pl.ds((s % per) * SEG, SEG), pl.ds(D, D)], s_out.at[1])

    def step(s, _):
        r0 = pl.multiple_of(s * SEG, SEG)
        hbuf[pl.ds(M, SEG), :] = xb[pl.ds(r0, SEG), :].astype(F32)
        row = lax.broadcasted_iota(jnp.int32, (L, 128), 0)
        col = lax.broadcasted_iota(jnp.int32, (L, 128), 1)
        keep = (col < L) & ((row < M) | (row >= col))
        fill = jnp.where(col < L, -1e9, -jnp.inf).astype(F32)
        zpad = jnp.zeros((128 - L, 128), F32)

        def proj(i, h):
            slot = h // 2 + (h % 2) * HP
            return _dot(hbuf[...], pltpu.bitcast(wqkv[i, slot], BF16))

        def scores(q, k):
            kp = jnp.concatenate([k, zpad], axis=0).astype(BF16)
            sc = jnp.where(keep, _dot(q, kp, NT) * scale, fill)
            e = jnp.exp(sc - jnp.max(sc, axis=1, keepdims=True))
            return e, 1.0 / jnp.sum(e, axis=1, keepdims=True)

        def pv(h, e, rcp, v):
            vp = jnp.concatenate([v, zpad], axis=0).astype(BF16)
            obuf[:, pl.ds(h * 128, 128)] = _dot(e, vp) * rcp

        qs, ks, vs, es = {}, {}, {}, {}
        for h in range(H + 2):
            if h < H:
                qs[h] = proj(0, h)
                ks[h] = proj(1, h)
            if 1 <= h <= H:
                es[h - 1] = scores(qs.pop(h - 1), ks.pop(h - 1))
                vs[h - 1] = proj(2, h - 1)
            if h >= 2:
                pv(h - 2, *es.pop(h - 2), vs.pop(h - 2))
        out = _dot(obuf[...], pltpu.bitcast(wo[...], BF16))
        hbuf[pl.ds(0, M), :] = out[:M]
        yb[pl.ds(r0, SEG), :] = out[M:]
        yb_copy(s).start()

    lax.fori_loop(0, NSEG, step, None)

    for b in range(NB):
        for c in range(NC):
            ya_copy(b, c).wait()
    for s in range(NSEG):
        yb_copy(s).wait()


@functools.partial(jax.jit, static_argnames=("B_seg_len",))
def pallas_concat_heads__ssm_conv_s5__memory_aug_recurrent_mem_tr__prompt_kernel(
    A_x, A_Lambda_re, A_Lambda_im, A_B_re, A_B_im, A_C_re, A_C_im, A_log_dt, A_Dskip,
    B_x, B_mem0, B_Wq, B_Wk, B_Wv, B_Wo, B_seg_len,
):
    _, S, D = A_x.shape
    _, H, Dh = B_Wq.shape
    M = B_mem0.shape[1]
    SEG = int(B_seg_len)
    LC = S // NC
    hbm = pl.BlockSpec(memory_space=pl.ANY)
    vmem = pl.BlockSpec(memory_space=pltpu.VMEM)
    row = lambda v: v.reshape(1, D)
    wview = lambda w: w.reshape(D // 2, 2 * H, Dh)
    out = pl.pallas_call(
        functools.partial(_kernel, S=S, D=D, H=H, M=M, SEG=SEG),
        out_shape=jax.ShapeDtypeStruct((NC, LC, 2 * D), F32),
        in_specs=[hbm, vmem, vmem, hbm, hbm, hbm, hbm, vmem, vmem,
                  hbm, vmem, hbm, hbm, hbm, hbm],
        out_specs=hbm,
        scratch_shapes=[
            pltpu.VMEM((LC // 2, NC, D), U32),
            pltpu.VMEM((2, D // 2, D), U32),
            pltpu.VMEM((2, D // 2, D), U32),
            pltpu.VMEM((2, LC, NC, D), F32),
            pltpu.VMEM((LC, NC, D), F32),
            pltpu.VMEM((7, NC, D), F32),
            pltpu.VMEM((S, D), BF16),
            pltpu.VMEM((3, H, D // 2, Dh), U32),
            pltpu.VMEM((H * Dh // 2, D), U32),
            pltpu.VMEM((S, D), F32),
            pltpu.VMEM((M + SEG, D), F32),
            pltpu.VMEM((M + SEG, H * Dh), F32),
            pltpu.SemaphoreType.DMA((LC // TB,)),
            pltpu.SemaphoreType.DMA((4,)),
            pltpu.SemaphoreType.DMA((3,)),
            pltpu.SemaphoreType.DMA((2,)),
            pltpu.SemaphoreType.DMA((2,)),
        ],
        compiler_params=pltpu.CompilerParams(vmem_limit_bytes=110 * 1024 * 1024),
    )(A_x.reshape(NC, LC, D), row(A_Lambda_re), row(A_Lambda_im), A_B_re, A_B_im, A_C_re, A_C_im,
      row(A_log_dt), row(A_Dskip), B_x.reshape(S, D), B_mem0.reshape(M, D),
      wview(B_Wq), wview(B_Wk), wview(B_Wv), B_Wo.reshape(H * Dh, D))
    return out.reshape(1, S, 2 * D)
```

```python
import functools

import jax
import jax.numpy as jnp
import numpy as np
from jax import lax
import jax.experimental.pallas as pl
import jax.experimental.pallas.tpu as pltpu

F32 = jnp.float32
BF16 = jnp.bfloat16
U32 = jnp.uint32
HI16 = np.uint32(0xFFFF0000)
LO16 = np.uint32(0x0000FFFF)
NT = (((1,), (1,)), ((), ()))
NN = (((1,), (0,)), ((), ()))

T = 128
NC = 8
NB = 4


def _dot(a, b, dims=NN):
    return lax.dot_general(a, b, dims, preferred_element_type=F32)


def _lanes(n):
    return pl.ds(n * T, T)


def _join(lists):
    return [x for l in lists for x in l]


def _start(copies):
    for cp in copies:
        cp.start()


def _wait(copies):
    for cp in copies:
        cp.wait()


def _cfma(ar, ai, br, bi, cr, ci):
    return (lax.add(lax.sub(lax.mul(ar, br), lax.mul(ai, bi)), cr),
            lax.add(lax.add(lax.mul(ar, bi), lax.mul(ai, br)), ci))


def _sum(terms):
    s, v = terms[0]
    for t, w in terms[1:]:
        if s == t:
            v = lax.add(w, v)
        else:
            s, v = 1, (lax.sub(v, w) if s > 0 else lax.sub(w, v))
    return s, v


class _Weaver:
    def __init__(self, ticks, tasks):
        self.total = sum(n for _, n in tasks)
        self.stream = (y for gen, _ in tasks for y in gen)
        self.ticks, self.now, self.done = ticks, 0, 0

    def tick(self):
        self.now += 1
        while self.done < self.total * min(self.now, self.ticks) // self.ticks:
            next(self.stream)
            self.done += 1
        if self.now == self.ticks:
            assert not list(self.stream)


_SA = (((1, 0), (1, 3)), ((1, 2), (1, 3)), ((1, 0),), ((1, 3),), ((1, 0), (1, 1)),
       ((1, 2), (-1, 0)), ((1, 1), (-1, 3)))
_SB = (((1, 0), (1, 3)), ((1, 0),), ((1, 1), (-1, 3)), ((1, 2), (-1, 0)), ((1, 3),),
       ((1, 0), (1, 1)), ((1, 2), (1, 3)))
_SC = (((1, 0), (1, 3), (-1, 4), (1, 6)), ((1, 2), (1, 4)), ((1, 1), (1, 3)),
       ((1, 0), (-1, 1), (1, 2), (1, 5)))


def _comb(terms, vals):
    return _sum([(s, vals[q]) for s, q in terms])[1]


def _block(outer, inner):
    return 2 * (outer // 2) + inner // 2, 2 * (outer % 2) + inner % 2


def _expand(tab, get, dst, slot, row, outer=range(7)):
    blk = [[get(*_block(o, i)) for o in range(4)] for i in range(4)]
    for j in outer:
        t = [_comb(tab[j], blk[i]) for i in range(4)]
        for k in range(7):
            dst[slot, 7 * j + k, pl.ds(row, 16), :] = _comb(tab[k], t).astype(BF16)
            if k in (3, 6):
                yield


def _collapse(src, row, out):
    for j in range(7):
        m = [src[7 * j + k, pl.ds(row, 8), :] for k in range(7)]
        t = [_comb(_SC[i], m) for i in range(4)]
        for o in range(4):
            for sign, jj in _SC[o]:
                if jj == j:
                    for i in range(4):
                        key = _block(o, i)
                        out[key] = _sum([(1, out[key]), (sign, t[i])])[1] if key in out else t[i]
        yield


def _hopcroft_kerr(n):
    lhs, steps, node = [], [], {}

    def product(*forms):
        lhs.append({(k, c % 3): s * v for s, a, c in forms for k, v in a.items()})
        return len(lhs) - 1

    def pair(i, j, via):
        if (node[i][0] - node[j][0]) % 3 != 1:
            i, j = j, i
        (ci, ai, bi, pi, qi), (cj, aj, bj, pj, qj) = node[i], node[j]
        av = {**aj, **{k: -v for k, v in ai.items()}}
        m = product((1, ai, cj), (1, aj, ci))
        p = product((1, av, cj))
        q = product((-1, av, ci))
        node[i, j] = node[j, i] = ((cj + 2) % 3, av, bi + bj, p, q)
        steps.append((m, p, q, cj, bi, bj, (pi, qi, pj, qj), via))

    for k in range(n):
        p, q = product((1, {k: 1}, k + 1)), product((-1, {k: 1}, k + 2))
        node[k] = (k % 3, {k: 1}, (k,), p, q)
        steps.append((p, q, k))
        for i in range(k):
            if (k - i) % 3:
                pair(i, k, None)
        for i in range(k):
            if (k - i) % 3 == 0:
                pair((i, i + 1), k, (i, i + 1, k, node[i, i + 1][1][i]))
    return steps, lhs


_HK_STEPS, _HK_LHS = _hopcroft_kerr(8)
_HK_SUMS = 68


def _hk_weights(get, put):
    cell, part = {}, {}

    def w(k, j):
        return _sum([(1, get(k, j))] + cell.pop((k, j), []))

    def add(r, s, v):
        part[r] = _sum([(s * v[0], v[1])] + ([part[r]] if r in part else []))

    for st in reversed(_HK_STEPS):
        if len(st) == 3:
            p, q, k = st
            v = w(k, k)
            add(p, 1, v)
            add(q, 1, v)
        else:
            m, p, q, _, bi, bj, (pi, qi, pj, qj), via = st
            if via is None:
                wij, wji = w(bi[0], bj[0]), w(bj[0], bi[0])
            else:
                i, j, k, s = via
                wik, wki = w(i, k), w(k, i)
                cell[j, k], cell[k, j] = [wik], [(-wki[0], wki[1])]
                wij, wji = (s * wik[0], wik[1]), wki
                if len(bi) == 1:
                    wij, wji = wji, wij
            put(m, _sum([wij, wji]))
            for r, s, v in ((q, -1, wij), (pj, 1, wij), (pi, -1, wij),
                            (p, 1, wji), (qi, 1, wji), (qj, -1, wji)):
                add(r, s, v)
        put(p, part.pop(p))
        put(q, part.pop(q))
        yield


def _hk_forms(x, y):
    y = y - 0.5 * x
    return (1, x), (1, y), (-1, x + y)


def _hk_accumulate(st, prod, acc):
    def add(j, g, s, v):
        if g % 3 == j % 3:
            add(j, g + 1, -s, v)
            add(j, g + 2, -s, v)
        else:
            acc[j, g % 3] = _sum([acc[j, g % 3], (s * v[0], v[1])])

    if len(st) == 3:
        p, q, k = st
        acc[k, (k + 2) % 3] = prod(p)
        acc[k, (k + 1) % 3] = prod(q)
    else:
        m, p, q, c, bi, bj = st[:6]
        m, p, q = prod(m), prod(p), prod(q)
        s = _sum([m, p, (-q[0], q[1])])
        for j in bi:
            add(j, c, -1, s)
            add(j, c + 2, -1, p)
        for j in bj:
            add(j, c + 1, 1, s)
            add(j, c + 2, -1, q)


def _hk_result(acc, j):
    def total(*terms):
        s, v = _sum([(s * acc[j, g][0], acc[j, g][1]) for s, g in terms if g != j % 3])
        return v if s > 0 else -v
    x = total((1, 1), (-1, 2))
    return x, total((1, 2), (-1, 0)) + 0.5 * x


def _s5(xa_hbm, vec_hbm, b_hbm, c_hbm, ya, wqkv, w_cp, late_cp, fence,
        vec, xa, braw, craw, u, par, lop0, lop1, rop0, rop1, rop2, pb0, pb1, pb2, pb3,
        s_vec, s_first, s_xa, s_b, s_c):
    D = xa.shape[-1]
    TB = 2 * xa.shape[1]
    NP = TB // 4
    pbs, lops, b_ops, c_ops = (pb0, pb1, pb2, pb3), (lop0, lop1), (rop0, rop1), (rop2, rop0)

    def products(pb, lop, rop, r0, tiles):
        def one(n):
            a, b = (jnp.concatenate([pltpu.bitcast(ref.bitcast(U32)[t0 + t, n], BF16) for t in tiles],
                                    axis=1) for ref, t0 in ((lop, 0), (rop, r0)))
            pb[n] = _dot(a, b, NT) + pb[n] if tiles[0] else _dot(a, b, NT)
        return [functools.partial(one, n) for n in range(49)]

    def x_copies(b, cols, sem):
        return [pltpu.make_async_copy(xa_hbm.bitcast(U32).at[b, c, :, cols], xa.at[b, :, c, cols], sem)
                for c in range(NC)]

    def w_copies(srcs, dst, rows, cols, sem):
        return [pltpu.make_async_copy(src.at[rows, cols], dst.at[z, rows, cols], sem)
                for z, src in enumerate(srcs)]

    full = pl.ds(0, D)
    xa_cp = [x_copies(b, full, s_xa.at[b]) for b in range(NB)]
    b_cp = [w_copies(b_hbm, braw, pl.ds(g * D // 4, D // 4), full, s_b.at[g]) for g in range(4)]
    c_cp = [w_copies(c_hbm, craw, pl.ds(g * D // 2, D // 2), full, s_c.at[g]) for g in range(2)]
    x0_cp, b0_cp = zip(*[
        (x_copies(0, cols, s_first.at[t]),
         w_copies(b_hbm, braw, pl.ds(0, D // 4), cols, s_first.at[2 + t]))
        for t, cols in enumerate((pl.ds(0, D // 2), pl.ds(D // 2, D // 2)))])
    vec_cp = [pltpu.make_async_copy(src, vec.at[i], s_vec) for i, src in enumerate(vec_hbm)]
    _start(vec_cp + x0_cp[0] + b0_cp[0] + x0_cp[1] + b0_cp[1] + b_cp[1])
    _wait(vec_cp)

    lre, lim, log_dt, dskip = (vec[i].astype(F32) for i in range(4))
    dt = jnp.exp(log_dt).astype(BF16).astype(F32)
    mag = jnp.exp(dt * lre)
    ar = mag * jnp.cos(dt * lim)
    ai = mag * jnp.sin(dt * lim)
    den = lre * lre + lim * lim
    vals = [2.0 * ((ar - 1.0) * lre + ai * lim) / den, -2.0 * (ai * lre - (ar - 1.0) * lim) / den]
    n = 1
    while n <= 4 * TB:
        if n in (1, 4, TB, 2 * TB, 4 * TB):
            vals += [ar, ai]
        ar, ai = ar * ar - ai * ai, 2.0 * ar * ai
        n *= 2
    G, LAM, LAM4, LAMT, DSK, END, RUN, INI = 0, 2, 4, 6, 12, 13, 15, 17
    for i, v in enumerate(vals + [dskip]):
        for n in range(D // T):
            par[i, :, _lanes(n)] = jnp.broadcast_to(v[n:n + 1], (NC, T))
    par[END] = jnp.zeros((NC, D), F32)
    par[END + 1] = jnp.zeros((NC, D), F32)

    def cplx(i, n):
        return par[i, :, _lanes(n)], par[i + 1, :, _lanes(n)]

    def put_cplx(i, n, v):
        par[i, :, _lanes(n)], par[i + 1, :, _lanes(n)] = v

    def x_at(b, p, q, n):
        w = xa[b, 2 * p + q // 2, :, _lanes(n)]
        return pltpu.bitcast(w & HI16 if q % 2 else w << 16, F32)

    def x_lhs(b, t):
        return [(_expand(_SA, lambda q, kb, p=p: jnp.concatenate(
            [x_at(b, p + i, q, 4 * t + kb) for i in range(2)], axis=0),
            lops[b % 2], t, p * NC), 14) for p in range(0, NP, 2)]

    def b_rhs(g, tiles=(0, 1), outer=range(7)):
        return [(_expand(_SB, lambda kb, nb, t=t, r=r: braw[
            nb % 2, pl.ds((2 * g + nb // 2) * T + r, 16), _lanes(4 * t + kb)].astype(F32),
            b_ops[g // 2], 2 * (g % 2) + t, r, outer), 2 * len(outer))
            for t in tiles for r in range(0, T, 16)]

    def u_post(b, g):
        def task(p):
            c = {}
            yield from _collapse(pbs[g], p * NC, c)
            for e in range(2):
                n = 2 * g + e
                for q in range(4):
                    v = c[q, 2 * e], c[q, 2 * e + 1]
                    u[b, n, 4 * p + q] = jnp.concatenate(v, axis=0).astype(BF16)
                    acc = v if q == 0 else _cfma(*cplx(LAM, n), *acc, *v)
                    if q == 3:
                        put_cplx(RUN, n, _cfma(*cplx(LAM4, n), *cplx(RUN, n), *acc) if p else acc)
                    if q % 2:
                        yield

        def carry(n):
            sub = lax.broadcasted_iota(jnp.int32, (NC, T), 0)
            run = cplx(RUN, n)
            ini = [pltpu.roll(jnp.where(sub == NC - 1, e, r), 1, 0) for e, r in zip(cplx(END, n), run)]
            for i in range(3):
                ini = _cfma(*cplx(LAMT + 2 * i, n),
                            *[jnp.where(sub >= 2 ** i, pltpu.roll(v, 2 ** i, 0), 0.0) for v in ini],
                            *ini)
            put_cplx(INI + 2 * b, n, ini)
            put_cplx(END, n, _cfma(*cplx(LAMT, n), *ini, *run))
            yield
        return [(task(p), 11) for p in range(NP)] + [(carry(2 * g + e), 1) for e in range(2)]

    def h_lhs(b):
        def task(t, p):
            hs = {}
            st = [cplx(INI + 2 * b, 2 * t + e) for e in range(2)]
            for i in range(4 * p, 4 * p + 8):
                for e in range(2):
                    v = u[b, 2 * t + e, i].astype(F32)
                    st[e] = _cfma(*cplx(LAM, 2 * t + e), *st[e], v[:NC], v[NC:])
                    for z in range(2):
                        hs.setdefault((i % 4, 2 * e + z), []).append(st[e][z])
                yield
            for e in range(2):
                put_cplx(INI + 2 * b, 2 * t + e, st[e])
            yield from _expand(_SA, lambda q, kb: jnp.concatenate(hs[q, kb], axis=0),
                               lops[b % 2], t, p * NC)
        return [(task(t, p), 22) for t in reversed(range(4)) for p in range(0, NP, 2)]

    def c_rhs(g):
        def task(t, r):
            blk = {}
            for e in range(2):
                gr, gi = (jnp.concatenate([v, v], axis=0) for v in cplx(G, 2 * t + e))
                for nb in range(4):
                    cr, ci = (craw[z, pl.ds((4 * g + nb) * T + r, 16), _lanes(2 * t + e)].astype(F32)
                              for z in range(2))
                    blk[2 * e, nb] = lax.add(lax.mul(gr, cr), lax.mul(gi, ci))
                    blk[2 * e + 1, nb] = lax.sub(lax.mul(gi, cr), lax.mul(gr, ci))
                    if nb % 2:
                        yield
            yield from _expand(_SB, lambda kb, nb: blk[kb, nb], c_ops[g], t, r)
        return [(task(t, r), 18) for t in range(4) for r in range(0, T, 16)]

    def y_post(b, g):
        def task(p):
            c = {}
            yield from _collapse(pbs[2 * (b % 2) + g], p * NC, c)
            for q in range(4):
                for nb in range(4):
                    n = 4 * g + nb
                    ya[b, 4 * p + q, :, _lanes(n)] = lax.add(
                        c[q, nb], lax.mul(x_at(b, p, q, n), par[DSK, :, _lanes(n)]))
                yield
        return [(task(p), 11) for p in range(NP)]

    def unzip(groups):
        w32 = wqkv.bitcast(U32)

        def task(p, r):
            e, o = w32[2 * p, pl.ds(r, 32)], w32[2 * p + 1, pl.ds(r, 32)]
            w32[2 * p, pl.ds(r, 32)] = (e & LO16) | (o << 16)
            w32[2 * p + 1, pl.ds(r, 32)] = (e >> 16) | (o & HI16)
            yield
        return [(task(p, r), 1)
                for c in groups for p in range(4 * c, 4 * c + 4) for r in range(0, D // 2, 32)]

    def xb_mm(b, g, tiles=(0, 1)):
        return products(pbs[g], lops[b % 2], b_ops[g // 2], 2 * (g % 2), tiles)

    def hc_mm(b, g):
        return products(pbs[2 * (b % 2) + g], lops[b % 2], c_ops[g], 0, range(4))

    mm = xb_mm(0, 0, (0,)) + xb_mm(0, 0, (1,)) + _join(xb_mm(0, g) for g in (1, 2, 3))
    xb2 = lambda b, g: xb_mm(b, g) + xb_mm(b, g + 1)
    post2 = lambda b, g: u_post(b, g) + u_post(b, g + 1)
    h0, h1, c0, c1 = h_lhs(0), h_lhs(1), c_rhs(0), c_rhs(1)
    for wait, start, main, tasks in (
            (x0_cp[0], b_cp[2], [], x_lhs(0, 0)),
            (b0_cp[0], b_cp[3], [], b_rhs(0, (0,))),
            ([], [], mm[:24], []),
            (x0_cp[1], [], mm[24:49], x_lhs(0, 1)),
            (b0_cp[1], [], [], b_rhs(0, (1,))),
            ([], [], mm[49:98], []),
            (b_cp[1], xa_cp[1], [], b_rhs(1, outer=range(3))),
            ([], [], mm[98:118], b_rhs(1, outer=range(3, 7))),
            (b_cp[2], xa_cp[2], mm[118:147], b_rhs(2)),
            (b_cp[3], c_cp[0], mm[147:195], b_rhs(3) + u_post(0, 0)),
            (xa_cp[1], xa_cp[3], mm[195:], x_lhs(1, 0) + x_lhs(1, 1) + u_post(0, 1)),
            (xa_cp[2], w_cp[0], xb2(1, 0), post2(0, 2) + x_lhs(2, 0) + x_lhs(2, 1)),
            (c_cp[0], _join(w_cp[1:3]), xb2(1, 2), post2(1, 0) + c0[:14] + h0[:6]),
            (xa_cp[3], c_cp[1], xb2(2, 0), post2(1, 2) + x_lhs(3, 0) + c0[14:22] + h0[6:12]),
            ([], _join(w_cp[3:5]), xb2(2, 2), post2(2, 0) + x_lhs(3, 1) + c0[22:] + h0[12:16]),
            ([], w_cp[5], xb2(3, 0), post2(2, 2) + h0[16:] + h1[:3]),
            (c_cp[1], _join(w_cp[6:8]), xb2(3, 2), post2(3, 0) + c1[:20]),
            ([], w_cp[8], hc_mm(0, 0), post2(3, 2) + c1[20:] + h1[3:8]),
            ([], _join(w_cp[9:11]), hc_mm(0, 1), y_post(0, 0) + h1[8:]),
            (_join(w_cp[:2]), w_cp[11] + late_cp[0], hc_mm(1, 0) + hc_mm(1, 1),
             y_post(0, 1) + h_lhs(2) + unzip(range(2))),
            (_join(w_cp[2:4]), _join(late_cp[1:3]), hc_mm(2, 0) + hc_mm(2, 1),
             y_post(1, 0) + y_post(1, 1) + h_lhs(3) + unzip(range(2, 4))),
            (_join(w_cp[4:8]), late_cp[3], hc_mm(3, 0),
             y_post(2, 0) + y_post(2, 1) + unzip(range(4, 8))),
            (_join(w_cp[8:]), [], hc_mm(3, 1), y_post(3, 0) + unzip(range(8, 12))),
            ([], [], [], y_post(3, 1))):
        _wait(wait)
        _start(start)
        fence()
        weaver = _Weaver(max(len(main) - len(main) // 49, 1), tasks)
        for product in main:
            product()
            weaver.tick()
        weaver.tick()
        fence()


def _transformer(mem0, out_hbm, wqkv, wo, xb, ya_cp, fence, wsum, wosum, pre, opre, yb, mem, s_yb):
    M, D = mem.shape
    NTL, NSEG, SEG, _ = xb.shape
    H = wqkv.shape[0] // 3
    L = M + SEG
    R = SEG
    G = 4
    NG = H // G
    per = yb.shape[2] // SEG
    scale = float(T) ** -0.5
    place = {}

    def yb_cp(it):
        return pltpu.make_async_copy(
            yb.at[it], out_hbm.at[pl.ds(it * yb.shape[1], yb.shape[1]), :, pl.ds(D, D)], s_yb)

    def put_rows(it, seg, row, n, v):
        r = (seg % per) * SEG
        r = r if isinstance(r, int) else pl.multiple_of(r, SEG)
        yb[it, seg // per, pl.ds(r + row, v.shape[0]), _lanes(n)] = v

    def weight_sums(src, dst, square, r):
        blocks = {}

        def get(k, j):
            blocks[k, j] = src(k, j, r).astype(F32)
            return blocks[k, j]

        def put(i, v):
            plain = [kj for kj, w in blocks.items() if w is v[1]]
            if i not in place:
                place[i] = (v[0], plain[0] if plain else
                            sum(isinstance(p[1], int) for p in place.values()))
            if not plain:
                dst[square, place[i][1], pl.ds(r, 16), :] = v[1].astype(BF16)
        return _hk_weights(get, put), len(_HK_STEPS)

    def sum_tasks(c):
        squares = [(lambda k, j, r, i=i: wqkv[i * H + 8 * c + j, pl.ds(k * T + r, 16), :],
                    wsum, 4 * i + c) for i in range(3)]
        squares.append((lambda k, j, r: wo[j, G * k + c, pl.ds(r, 16), :], wosum, c))
        return [weight_sums(*sq, r) for r in range(0, T, 16) for sq in squares]

    def xrows(s, i):
        return jnp.concatenate([xb[n, s, pl.ds(M * i, M), :].astype(F32) for n in range(NTL)], axis=1)

    def w_in(i, hd, k0, nk):
        return pltpu.bitcast(wqkv.bitcast(U32)[i * H + hd, pl.ds(k0 * T // 2, nk * T // 2), :], BF16)

    def w_out(c, n):
        return pltpu.bitcast(wo.bitcast(U32)[n, pl.ds(G * c, G)].reshape(G * T // 2, T), BF16)

    def step(it, seg, phase):
        s = 4 * it + seg
        row = lax.broadcasted_iota(jnp.int32, (L, T), 0)
        col = lax.broadcasted_iota(jnp.int32, (L, T), 1)
        pos = lambda i: jnp.where(i < M, i, jnp.where(i < R, i + M, i - (R - M)))
        keep = (col < L) & ((row < M) | (pos(row) >= pos(col)))
        fill = jnp.where(col < L, -1e9, -jnp.inf).astype(F32)
        zpad = jnp.zeros((T - L, T), F32)
        tick = lambda: None

        if phase is None:
            tick = _Weaver(4 * H - 2, sum_tasks(s)).tick
            h = jnp.concatenate([mem[...]] + [xrows(s, i) for i in (1, 2, 3, 0)], axis=0)

            def proj(i, hd):
                v = _dot(h, w_in(i, hd, 0, NTL))
                tick()
                return v
        elif phase == 0:
            forms = _hk_forms(jnp.concatenate([mem[...]] + [xrows(s, i) for i in (1, 2, 3)], axis=0),
                              jnp.concatenate([xrows(s + i, 0) for i in range(4)], axis=0))
            lhs, done = {}, {}

            def square(i, c):
                def prod(r):
                    if r not in lhs:
                        sg, v = _sum([(t * forms[f][0], forms[f][1][:, k * T:(k + 1) * T])
                                      for (k, f), t in _HK_LHS[r].items()])
                        lhs[r] = sg, v.astype(BF16)
                    sg, at = place[r]
                    w = (pltpu.bitcast(wsum.bitcast(U32)[4 * i + c, at], BF16) if isinstance(at, int)
                         else w_in(i, 8 * c + at[1], at[0], 1))
                    return sg * lhs[r][0], _dot(lhs[r][1], w)
                acc = {}
                for st in _HK_STEPS:
                    _hk_accumulate(st, prod, acc)
                for j in range(0, 8, 2):
                    res = [_hk_result(acc, j + e) for e in range(2)]
                    for e in range(2):
                        done[i, 8 * c + j + e] = jnp.concatenate([res[e][0], res[e][1][:M]], axis=0)
                    for v in range(1, 4):
                        pre[(i * H + 8 * c + j) // 2, v - 1] = jnp.concatenate(
                            [y[M * v:M * v + M] for _, y in res], axis=0).astype(BF16)

            def proj(i, hd):
                if (i, hd) not in done:
                    square(i, hd // 8)
                return done[i, hd]
        else:
            h = jnp.concatenate([
                jnp.concatenate([mem[...], xrows(s, 1)], axis=0).astype(BF16),
                jnp.concatenate([pltpu.bitcast(xb.bitcast(U32)[n, s, pl.ds(M, M), :], BF16)
                                 for n in range(NTL)], axis=1)], axis=0)
            low = {(i, hd): _dot(h[:, :D // 2], w_in(i, hd, 0, NTL // 2))
                   for hd in range(2) for i in range(2)}

            def proj(i, hd):
                v = (_dot(h[:, D // 2:], w_in(i, hd, NTL // 2, NTL // 2)) + low[i, hd]
                     if (i, hd) in low else _dot(h, w_in(i, hd, 0, NTL)))
                first = pre[(i * H + hd) // 2, phase - 1].astype(F32)[M * (hd % 2):M * (hd % 2) + M]
                return jnp.concatenate([v, first], axis=0)

        def pad(v):
            return jnp.concatenate([v, zpad], axis=0).astype(BF16)

        def heads(g):
            return range(g * G, g * G + G) if 0 <= g < NG else ()

        lag_s, lag_pv, lag_o = {0: (2, 4, 5), 3: (1, 2, 4)}.get(phase, (1, 2, 3))
        qs, ks, vs, es, os, oforms, acc = {}, {}, {}, {}, {}, {}, {}
        todo = list(_HK_STEPS)
        for g in range(NG + lag_o):
            for hd in heads(g):
                qs[hd] = proj(0, hd)
                ks[hd] = proj(1, hd)
            for hd in heads(g - lag_s):
                sc = jnp.where(keep, _dot(qs[hd], pad(ks[hd]), NT) * scale, fill)
                e = jnp.exp(sc - jnp.max(sc, axis=1, keepdims=True))
                es[hd] = e, pltpu.reciprocal(jnp.sum(e, axis=1, keepdims=True), full_range=False)
            for hd in heads(g - lag_s):
                vs[hd] = proj(2, hd)
            for hd in heads(g - lag_pv):
                o = _dot(es[hd][0], pad(vs[hd])) * es[hd][1]
                if phase in (None, 3):
                    os[hd] = o
                else:
                    os[hd] = o[:R].astype(BF16)
                    opre[phase, :, _lanes(hd)] = o[R:]
            c = g - lag_o
            if c < 0:
                continue
            o = jnp.concatenate([os[hd] for hd in heads(c)], axis=1)
            if phase == 3:
                late = opre[:, :, pl.ds(c * G * T, G * T)].reshape(3 * M, G * T)
                oforms[c] = _hk_forms(o[:R], jnp.concatenate([o[R:], late], axis=0))

                def prod(r):
                    sg, v = _sum([(t * oforms[k][f][0], oforms[k][f][1])
                                  for (k, f), t in _HK_LHS[r].items()])
                    at = place[r][1]
                    w = (pltpu.bitcast(wosum.bitcast(U32)[:, at].reshape(G * T // 2, T), BF16)
                         if isinstance(at, int) else w_out(*at))
                    return sg * place[r][0], _dot(v.astype(BF16), w)
                for _ in range(c + 1):
                    _hk_accumulate(todo.pop(0), prod, acc)
            else:
                for n in range(NTL):
                    part = _dot(o, w_out(c, n))
                    acc[n] = part + acc[n] if c else part
                    if n % 2:
                        tick()
        for n in range(NTL):
            if phase == 3:
                out, late = _hk_result(acc, n)
                for v in range(4):
                    put_rows(it, (v + 3) % 4, 0, n, late[M * v:M * v + M])
            else:
                out = acc[n]
                if phase is None:
                    put_rows(it, seg, 0, n, out[R:])
            mem[:, _lanes(n)] = out[:M]
            put_rows(it, seg, M, n, out[M:R])

    def warm_up(seg, _):
        step(0, seg, None)
        fence()
        _start(ya_cp(seg))

    def four_steps(it, _):
        for phase in range(4):
            step(it, phase, phase)
        yb_cp(it).start()

    mem[...] = mem0[...].astype(F32)
    lax.fori_loop(0, 4, warm_up, None)
    yb_cp(0).start()
    lax.fori_loop(1, NSEG // 4, four_steps, None)
    _wait([yb_cp(it) for it in range(NSEG // 4)])


def _kernel(xa_hbm, lre_hbm, lim_hbm, bre_hbm, bim_hbm, cre_hbm, cim_hbm, ldt_hbm, dsk_hbm,
            xb_hbm, mem0_hbm, wq_hbm, wk_hbm, wv_hbm, wo_hbm, out_hbm,
            ya, xb, mem0, wqkv, wo, s_w, s_late, s_ya, s_fence):
    _, TB, _, D = ya.shape
    NTL, NSEG, SEG, _ = xb.shape
    H = wqkv.shape[0] // 3
    M = mem0.shape[0]

    def fence():
        pl.semaphore_signal(s_fence)
        pl.semaphore_wait(s_fence)

    w_cp = [[pltpu.make_async_copy(w.bitcast(U32).at[:, (hd % 2) * (H // 2) + hd // 2, :],
                                   wqkv.bitcast(U32).at[i * H + hd], s_w.at[(i * H + hd) // 8])
             for hd in range(c, c + 8)]
            for i, w in enumerate((wq_hbm, wk_hbm, wv_hbm)) for c in range(0, H, 8)]
    late_cp = [[pltpu.make_async_copy(src.at[:, :, _lanes(n)], dst.at[n], s_late)
                for n in range(c, c + 2) for src, dst in ((wo_hbm, wo), (xb_hbm, xb))]
               for c in range(0, NTL, 2)]
    late_cp[0].append(pltpu.make_async_copy(mem0_hbm, mem0, s_late))

    def ya_cp(b):
        return [pltpu.make_async_copy(ya.at[b, :, c, :], out_hbm.at[b * NC + c, :, pl.ds(0, D)], s_ya)
                for c in range(NC)]

    pl.run_scoped(
        functools.partial(_s5, xa_hbm, (lre_hbm, lim_hbm, ldt_hbm, dsk_hbm), (bre_hbm, bim_hbm),
                          (cre_hbm, cim_hbm), ya, wqkv, w_cp, late_cp, fence),
        pltpu.VMEM((4, NTL, T), BF16),
        pltpu.VMEM((NB, TB // 2, NC, D), U32),
        pltpu.VMEM((2, D, D), BF16),
        pltpu.VMEM((2, D, D), BF16),
        pltpu.VMEM((NB, NTL, TB, 2 * NC, T), BF16),
        pltpu.VMEM((17 + 2 * NB, NC, D), F32),
        *[pltpu.VMEM((4, 49, T, T), BF16)] * 5,
        *[pltpu.VMEM((49, T, T), F32)] * 4,
        pltpu.SemaphoreType.DMA,
        pltpu.SemaphoreType.DMA((4,)),
        pltpu.SemaphoreType.DMA((NB,)),
        pltpu.SemaphoreType.DMA((4,)),
        pltpu.SemaphoreType.DMA((2,)),
    )
    _wait(_join(late_cp))
    pl.run_scoped(
        functools.partial(_transformer, mem0, out_hbm, wqkv, wo, xb, ya_cp, fence),
        pltpu.VMEM((3 * H // 8, _HK_SUMS, T, T), BF16),
        pltpu.VMEM((4, _HK_SUMS, T, T), BF16),
        pltpu.VMEM((3 * H // 2, 3, 2 * M, T), BF16),
        pltpu.VMEM((3, M, H * T), F32),
        pltpu.VMEM((NSEG // 4, 4 * SEG // TB, TB, D), F32),
        pltpu.VMEM((M, D), F32),
        pltpu.SemaphoreType.DMA,
    )
    _wait(_join(ya_cp(b) for b in range(NB)))


@functools.partial(jax.jit, static_argnames=("B_seg_len",))
def pallas_concat_heads__ssm_conv_s5__memory_aug_recurrent_mem_tr__prompt_kernel(
    A_x, A_Lambda_re, A_Lambda_im, A_B_re, A_B_im, A_C_re, A_C_im, A_log_dt, A_Dskip,
    B_x, B_mem0, B_Wq, B_Wk, B_Wv, B_Wo, B_seg_len,
):
    _, S, D = A_x.shape
    _, H, Dh = B_Wq.shape
    M = B_mem0.shape[1]
    SEG = int(B_seg_len)
    TB = S // (NB * NC)
    assert (S, D, H, Dh, M, SEG) == (2048, 1024, 32, 128, 8, 32)
    hbm = pl.BlockSpec(memory_space=pl.ANY)
    tile = lambda v: v.reshape(D // T, T)
    pairs = lambda w: w.reshape(D // 2, 2 * H, Dh)
    out = pl.pallas_call(
        _kernel,
        out_shape=jax.ShapeDtypeStruct((NB * NC, TB, 2 * D), F32),
        in_specs=[hbm] * 15,
        out_specs=hbm,
        scratch_shapes=[
            pltpu.VMEM((NB, TB, NC, D), F32),
            pltpu.VMEM((D // T, S // SEG, SEG, T), BF16),
            pltpu.VMEM((M, D), BF16),
            pltpu.VMEM((3 * H, D, T), BF16),
            pltpu.VMEM((D // T, H, Dh, T), BF16),
            pltpu.SemaphoreType.DMA((3 * H // 8,)),
            pltpu.SemaphoreType.DMA,
            pltpu.SemaphoreType.DMA,
            pltpu.SemaphoreType.REGULAR,
        ],
        compiler_params=pltpu.CompilerParams(vmem_limit_bytes=116 * 1024 * 1024),
    )(A_x.reshape(NB, NC, TB, D), tile(A_Lambda_re), tile(A_Lambda_im),
      A_B_re, A_B_im, A_C_re, A_C_im, tile(A_log_dt), tile(A_Dskip),
      B_x.reshape(S // SEG, SEG, D), B_mem0.reshape(M, D),
      pairs(B_Wq), pairs(B_Wk), pairs(B_Wv), B_Wo)
    return out.reshape(1, S, 2 * D)
```

```python
import functools

import jax
import jax.numpy as jnp
import numpy as np
from jax import lax
import jax.experimental.pallas as pl
import jax.experimental.pallas.tpu as pltpu

F32 = jnp.float32
BF16 = jnp.bfloat16
U32 = jnp.uint32
HI16 = np.uint32(0xFFFF0000)
LO16 = np.uint32(0x0000FFFF)
NT = (((1,), (1,)), ((), ()))
NN = (((1,), (0,)), ((), ()))

T = 128
NC = 8
NB = 4


def _dot(a, b, dims=NN):
    return lax.dot_general(a, b, dims, preferred_element_type=F32)


def _lanes(n):
    return pl.ds(n * T, T)


def _join(lists):
    return [x for l in lists for x in l]


def _start(copies):
    for cp in copies:
        cp.start()


def _wait(copies):
    for cp in copies:
        cp.wait()


def _cfma(ar, ai, br, bi, cr, ci):
    return (lax.add(lax.sub(lax.mul(ar, br), lax.mul(ai, bi)), cr),
            lax.add(lax.add(lax.mul(ar, bi), lax.mul(ai, br)), ci))


def _sum(terms):
    s, v = terms[0]
    for t, w in terms[1:]:
        if s == t:
            v = lax.add(w, v)
        else:
            s, v = 1, (lax.sub(v, w) if s > 0 else lax.sub(w, v))
    return s, v


class _Weaver:
    def __init__(self, ticks, tasks):
        self.total = sum(n for _, n in tasks)
        self.stream = (y for gen, _ in tasks for y in gen)
        self.ticks, self.now, self.done = ticks, 0, 0

    def tick(self):
        self.now += 1
        while self.done < self.total * min(self.now, self.ticks) // self.ticks:
            next(self.stream)
            self.done += 1
        if self.now == self.ticks:
            assert not list(self.stream)


_SA = (((1, 0), (1, 3)), ((1, 2), (1, 3)), ((1, 0),), ((1, 3),), ((1, 0), (1, 1)),
       ((1, 2), (-1, 0)), ((1, 1), (-1, 3)))
_SB = (((1, 0), (1, 3)), ((1, 0),), ((1, 1), (-1, 3)), ((1, 2), (-1, 0)), ((1, 3),),
       ((1, 0), (1, 1)), ((1, 2), (1, 3)))
_SC = (((1, 0), (1, 3), (-1, 4), (1, 6)), ((1, 2), (1, 4)), ((1, 1), (1, 3)),
       ((1, 0), (-1, 1), (1, 2), (1, 5)))


def _comb(terms, vals):
    return _sum([(s, vals[q]) for s, q in terms])[1]


def _block(outer, inner):
    return 2 * (outer // 2) + inner // 2, 2 * (outer % 2) + inner % 2


def _expand(tab, get, dst, slot, row):
    blk = [[get(*_block(o, i)) for o in range(4)] for i in range(4)]
    for j in range(7):
        t = [_comb(tab[j], blk[i]) for i in range(4)]
        for k in range(7):
            dst[slot, 7 * j + k, pl.ds(row, 16), :] = _comb(tab[k], t).astype(BF16)
            if k in (3, 6):
                yield


def _collapse(src, row, out):
    for j in range(7):
        m = [src[7 * j + k, pl.ds(row, 8), :] for k in range(7)]
        t = [_comb(_SC[i], m) for i in range(4)]
        for o in range(4):
            for sign, jj in _SC[o]:
                if jj == j:
                    for i in range(4):
                        key = _block(o, i)
                        out[key] = _sum([(1, out[key]), (sign, t[i])])[1] if key in out else t[i]
        yield


def _hopcroft_kerr(n):
    lhs, steps, node = [], [], {}

    def product(*forms):
        lhs.append({(k, c % 3): s * v for s, a, c in forms for k, v in a.items()})
        return len(lhs) - 1

    def pair(i, j, via):
        if (node[i][0] - node[j][0]) % 3 != 1:
            i, j = j, i
        (ci, ai, bi, pi, qi), (cj, aj, bj, pj, qj) = node[i], node[j]
        av = {**aj, **{k: -v for k, v in ai.items()}}
        m = product((1, ai, cj), (1, aj, ci))
        p = product((1, av, cj))
        q = product((-1, av, ci))
        node[i, j] = node[j, i] = ((cj + 2) % 3, av, bi + bj, p, q)
        steps.append((m, p, q, cj, bi, bj, (pi, qi, pj, qj), via))

    for k in range(n):
        p, q = product((1, {k: 1}, k + 1)), product((-1, {k: 1}, k + 2))
        node[k] = (k % 3, {k: 1}, (k,), p, q)
        steps.append((p, q, k))
        for i in range(k):
            if (k - i) % 3:
                pair(i, k, None)
            else:
                pair((i, i + 1), k, (i, i + 1, k, node[i, i + 1][1][i]))
    return steps, lhs


_HK_STEPS, _HK_LHS = _hopcroft_kerr(8)
_HK_SUMS = 68


def _hk_weights(get, put):
    cell, part = {}, {}

    def w(k, j):
        return _sum([(1, get(k, j))] + cell.pop((k, j), []))

    def add(r, s, v):
        part[r] = _sum([(s * v[0], v[1])] + ([part[r]] if r in part else []))

    for st in sorted(_HK_STEPS, key=lambda st: (st[2], 2, 0) if len(st) == 3 else
                     (min(st[4] + st[5]), st[7] is None, max(st[4] + st[5]))):
        if len(st) == 3:
            p, q, k = st
            v = w(k, k)
            add(p, 1, v)
            add(q, 1, v)
        else:
            m, p, q, _, bi, bj, (pi, qi, pj, qj), via = st
            if via is None:
                wij, wji = w(bi[0], bj[0]), w(bj[0], bi[0])
            else:
                i, j, k, s = via
                wik, wki = w(i, k), w(k, i)
                cell[j, k], cell[k, j] = [wik], [(-wki[0], wki[1])]
                wij, wji = (s * wik[0], wik[1]), wki
                if len(bi) == 1:
                    wij, wji = wji, wij
            put(m, _sum([wij, wji]))
            for r, s, v in ((q, -1, wij), (pj, 1, wij), (pi, -1, wij),
                            (p, 1, wji), (qi, 1, wji), (qj, -1, wji)):
                add(r, s, v)
        put(p, part.pop(p))
        put(q, part.pop(q))
        yield


def _hk_forms(x, y):
    y = y - 0.5 * x
    return (1, x), (1, y), (-1, x + y)


def _hk_accumulate(st, prod, acc):
    def add(j, g, s, v):
        if g % 3 == j % 3:
            add(j, g + 1, -s, v)
            add(j, g + 2, -s, v)
        else:
            acc[j, g % 3] = _sum([acc[j, g % 3], (s * v[0], v[1])])

    if len(st) == 3:
        p, q, k = st
        acc[k, (k + 2) % 3] = prod(p)
        acc[k, (k + 1) % 3] = prod(q)
    else:
        m, p, q, c, bi, bj = st[:6]
        m, p, q = prod(m), prod(p), prod(q)
        s = _sum([m, p, (-q[0], q[1])])
        for j in bi:
            add(j, c, -1, s)
            add(j, c + 2, -1, p)
        for j in bj:
            add(j, c + 1, 1, s)
            add(j, c + 2, -1, q)


def _hk_result(acc, j):
    def total(*terms):
        s, v = _sum([(s * acc[j, g][0], acc[j, g][1]) for s, g in terms if g != j % 3])
        return v if s > 0 else -v
    x = total((1, 1), (-1, 2))
    return x, total((1, 2), (-1, 0)) + 0.5 * x


def _s5(xa_hbm, vec_hbm, b_hbm, c_hbm, ya, wqkv, w_cp, late_cp, fence,
        vec, xa, braw, craw, u, par, lop0, lop1, rop0, rop1, rop2, pb0, pb1, pb2, pb3,
        s_vec, s_xa, s_b, s_c):
    D = xa.shape[-1]
    TB = 2 * xa.shape[1]
    NP = TB // 4
    pbs, lops, b_ops, c_ops = (pb0, pb1, pb2, pb3), (lop0, lop1), (rop0, rop1), (rop2, rop0)

    def products(pb, lop, rop, r0, tiles):
        def one(n):
            a, b = (jnp.concatenate([pltpu.bitcast(ref.bitcast(U32)[t0 + t, n], BF16) for t in tiles],
                                    axis=1) for ref, t0 in ((lop, 0), (rop, r0)))
            pb[n] = _dot(a, b, NT) + pb[n] if tiles[0] else _dot(a, b, NT)
        return [functools.partial(one, n) for n in range(49)]

    def x_copies(b, cols, sem):
        return [pltpu.make_async_copy(xa_hbm.bitcast(U32).at[b, c, :, cols], xa.at[b, :, c, cols], sem)
                for c in range(NC)]

    def w_copies(srcs, dst, rows, cols, sem):
        return [pltpu.make_async_copy(src.at[rows, cols], dst.at[z, rows, cols], sem)
                for z, src in enumerate(srcs)]

    full, halves = pl.ds(0, D), (pl.ds(0, D // 2), pl.ds(D // 2, D // 2))
    x0_cp = [x_copies(0, cols, s_xa.at[NB * t]) for t, cols in enumerate(halves)]
    xa_cp = {b: x_copies(b, full, s_xa.at[b]) for b in range(1, NB)}
    b_cp = [w_copies(b_hbm, braw, pl.ds(g * D // 4, D // 4), cols, s_b.at[2 * g + t])
            for g in range(4) for t, cols in enumerate(halves)]
    c_cp = [w_copies(c_hbm, craw, pl.ds(g * D // 2, D // 2), full, s_c.at[g]) for g in range(2)]
    vec_cp = [pltpu.make_async_copy(src, vec.at[i], s_vec) for i, src in enumerate(vec_hbm)]
    _start(vec_cp + x0_cp[0] + b_cp[0] + b_cp[2] + x0_cp[1])
    _wait(vec_cp)

    lre, lim, log_dt, dskip = (vec[i].astype(F32) for i in range(4))
    dt = jnp.exp(log_dt).astype(BF16).astype(F32)
    mag = jnp.exp(dt * lre)
    ar = mag * jnp.cos(dt * lim)
    ai = mag * jnp.sin(dt * lim)
    den = lre * lre + lim * lim
    vals = [2.0 * ((ar - 1.0) * lre + ai * lim) / den, -2.0 * (ai * lre - (ar - 1.0) * lim) / den]
    n = 1
    while n <= 4 * TB:
        if n in (1, 4, TB, 2 * TB, 4 * TB):
            vals += [ar, -ai]
        ar, ai = ar * ar - ai * ai, 2.0 * ar * ai
        n *= 2
    G, LAM, LAM4, LAMT, DSK, END, RUN, INI = 0, 2, 4, 6, 12, 13, 15, 17
    for i, v in enumerate(vals + [dskip]):
        for n in range(D // T):
            par[i, :, _lanes(n)] = jnp.broadcast_to(v[n:n + 1], (NC, T))
    par[END] = jnp.zeros((NC, D), F32)
    par[END + 1] = jnp.zeros((NC, D), F32)

    def cplx(i, n):
        return par[i, :, _lanes(n)], par[i + 1, :, _lanes(n)]

    def put_cplx(i, n, v):
        par[i, :, _lanes(n)], par[i + 1, :, _lanes(n)] = v

    def x_at(b, p, q, n):
        w = xa[b, 2 * p + q // 2, :, _lanes(n)]
        return pltpu.bitcast(w & HI16 if q % 2 else w << 16, F32)

    def x_lhs(b, t):
        return [(_expand(_SA, lambda q, kb, p=p: jnp.concatenate(
            [x_at(b, p + i, q, 4 * t + kb) for i in range(2)], axis=0),
            lops[b % 2], t, p * NC), 14) for p in range(0, NP, 2)]

    def b_rhs(g, t):
        return [(_expand(_SB, lambda kb, nb, r=r: braw[
            nb % 2, pl.ds((2 * g + nb // 2) * T + r, 16), _lanes(4 * t + kb)].astype(F32),
            b_ops[g // 2], 2 * (g % 2) + t, r), 14) for r in range(0, T, 16)]

    def u_post(b, g):
        def task(p):
            c = {}
            yield from _collapse(pbs[g], p * NC, c)
            for e in range(2):
                n = 2 * g + e
                for q in range(4):
                    (gr, gi), vr, vi = cplx(G, n), c[q, 2 * e], c[q, 2 * e + 1]
                    v = (lax.add(lax.mul(gr, vr), lax.mul(gi, vi)),
                         lax.sub(lax.mul(gi, vr), lax.mul(gr, vi)))
                    u[b, n, 4 * p + q] = jnp.concatenate(v, axis=0).astype(BF16)
                    acc = v if q == 0 else _cfma(*cplx(LAM, n), *acc, *v)
                    if q == 3:
                        put_cplx(RUN, n, _cfma(*cplx(LAM4, n), *cplx(RUN, n), *acc) if p else acc)
                    yield

        def carry(n):
            sub = lax.broadcasted_iota(jnp.int32, (NC, T), 0)
            run = cplx(RUN, n)
            ini = [pltpu.roll(jnp.where(sub == NC - 1, e, r), 1, 0) for e, r in zip(cplx(END, n), run)]
            for i in range(3):
                ini = _cfma(*cplx(LAMT + 2 * i, n),
                            *[jnp.where(sub >= 2 ** i, pltpu.roll(v, 2 ** i, 0), 0.0) for v in ini],
                            *ini)
            put_cplx(INI + 2 * b, n, ini)
            put_cplx(END, n, _cfma(*cplx(LAMT, n), *ini, *run))
            yield
        return [(task(p), 15) for p in range(NP)] + [(carry(2 * g + e), 1) for e in range(2)]

    def h_lhs(b):
        def task(t, p):
            hs = {}
            st = [cplx(INI + 2 * b, 2 * t + e) for e in range(2)]
            for i in range(4 * p, 4 * p + 8):
                for e in range(2):
                    v = u[b, 2 * t + e, i].astype(F32)
                    st[e] = _cfma(*cplx(LAM, 2 * t + e), *st[e], v[:NC], v[NC:])
                    for z in range(2):
                        hs.setdefault((i % 4, 2 * e + z), []).append(st[e][z])
                yield
            for e in range(2):
                put_cplx(INI + 2 * b, 2 * t + e, st[e])
            yield from _expand(_SA, lambda q, kb: jnp.concatenate(hs[q, kb], axis=0),
                               lops[b % 2], t, p * NC)
        return [(task(t, p), 22) for t in reversed(range(4)) for p in range(0, NP, 2)]

    def c_rhs(g):
        return [(_expand(_SB, lambda kb, nb, t=t, r=r: craw[
            kb % 2, pl.ds((4 * g + nb) * T + r, 16), _lanes(2 * t + kb // 2)].astype(F32),
            c_ops[g], t, r), 14) for t in range(4) for r in range(0, T, 16)]

    def y_post(b, g):
        def task(p):
            c = {}
            yield from _collapse(pbs[2 * (b % 2) + g], p * NC, c)
            for q in range(4):
                for nb in range(4):
                    n = 4 * g + nb
                    ya[(b, *divmod(4 * p + q, ya.shape[2]), slice(None), _lanes(n))] = lax.add(
                        c[q, nb], lax.mul(x_at(b, p, q, n), par[DSK, :, _lanes(n)]))
                yield
        return [(task(p), 11) for p in range(NP)]

    def unzip(groups):
        w32 = wqkv.bitcast(U32)

        def task(p, r):
            e, o = w32[2 * p, pl.ds(r, 32)], w32[2 * p + 1, pl.ds(r, 32)]
            w32[2 * p, pl.ds(r, 32)] = (e & LO16) | (o << 16)
            w32[2 * p + 1, pl.ds(r, 32)] = (e >> 16) | (o & HI16)
            yield
        return [(task(p, r), 1)
                for c in groups for p in range(4 * c, 4 * c + 4) for r in range(0, D // 2, 32)]

    def xb_mm(b, g, tiles=(0, 1)):
        return products(pbs[g], lops[b % 2], b_ops[g // 2], 2 * (g % 2), tiles)

    def hc_mm(b, g):
        return products(pbs[2 * (b % 2) + g], lops[b % 2], c_ops[g], 0, range(4))

    mm = _join(xb_mm(0, g, (t,)) for t in range(2) for g in range(2)) + xb_mm(0, 2) + xb_mm(0, 3)
    xb2 = lambda b, g: xb_mm(b, g) + xb_mm(b, g + 1)
    post2 = lambda b, g: u_post(b, g) + u_post(b, g + 1)
    u0, h0, h1, c0, c1 = u_post(0, 0), h_lhs(0), h_lhs(1), c_rhs(0), c_rhs(1)
    for wait, start, main, tasks in (
            (x0_cp[0], b_cp[1] + b_cp[3], [], x_lhs(0, 0)),
            (b_cp[0], _join(b_cp[4:]), [], b_rhs(0, 0)),
            ([], [], mm[:24], []),
            (b_cp[2], [], mm[24:48], b_rhs(1, 0)),
            (x0_cp[1], [], mm[48:76], x_lhs(0, 1)),
            (b_cp[1], [], mm[76:96], b_rhs(0, 1)),
            (b_cp[3], xa_cp[1], mm[96:144], b_rhs(1, 1)),
            (b_cp[4], [], mm[144:172], b_rhs(2, 0)),
            (b_cp[5], xa_cp[2], mm[172:196], b_rhs(2, 1)),
            (b_cp[6], [], mm[196:220], b_rhs(3, 0) + u0[:8]),
            (b_cp[7], c_cp[0], mm[220:244], b_rhs(3, 1) + u0[8:]),
            (xa_cp[1], xa_cp[3], mm[244:], x_lhs(1, 0) + x_lhs(1, 1) + u_post(0, 1)),
            (xa_cp[2], w_cp[0], xb2(1, 0), post2(0, 2) + x_lhs(2, 0) + x_lhs(2, 1)),
            (c_cp[0], _join(w_cp[1:3]), xb2(1, 2), post2(1, 0) + c0[:14] + h0[:6]),
            (xa_cp[3], c_cp[1], xb2(2, 0), post2(1, 2) + x_lhs(3, 0) + c0[14:22] + h0[6:12]),
            ([], _join(w_cp[3:5]), xb2(2, 2), post2(2, 0) + x_lhs(3, 1) + c0[22:] + h0[12:16]),
            ([], w_cp[5], xb2(3, 0), post2(2, 2) + h0[16:] + h1[:3]),
            (c_cp[1], _join(w_cp[6:8]), xb2(3, 2), post2(3, 0) + c1[:20]),
            ([], w_cp[8], hc_mm(0, 0), post2(3, 2) + c1[20:] + h1[3:8]),
            ([], _join(w_cp[9:11]), hc_mm(0, 1), y_post(0, 0) + h1[8:]),
            (_join(w_cp[:2]), w_cp[11] + late_cp[0], hc_mm(1, 0) + hc_mm(1, 1),
             y_post(0, 1) + h_lhs(2) + unzip(range(2))),
            (_join(w_cp[2:4]), _join(late_cp[1:3]), hc_mm(2, 0) + hc_mm(2, 1),
             y_post(1, 0) + y_post(1, 1) + h_lhs(3) + unzip(range(2, 4))),
            (_join(w_cp[4:8]), late_cp[3], hc_mm(3, 0),
             y_post(2, 0) + y_post(2, 1) + unzip(range(4, 8))),
            (_join(w_cp[8:]), [], hc_mm(3, 1), y_post(3, 0) + unzip(range(8, 12))),
            ([], [], [], y_post(3, 1))):
        _wait(wait)
        _start(start)
        fence()
        weaver = _Weaver(max(len(main) - len(main) // 49, 1), tasks)
        for product in main:
            product()
            weaver.tick()
        weaver.tick()
        fence()


def _transformer(mem0, out_hbm, wqkv, wo, xb, ya_cp, fence, wsum, wosum, pre, opre, yb, mem, s_yb):
    M, D = mem.shape
    NTL, NSEG, SEG, _ = xb.shape
    H = wqkv.shape[0] // 3
    L = M + SEG
    R = SEG
    G = 4
    NG = H // G
    _, CPG, SPC, _, _ = yb.shape
    scale = float(T) ** -0.5
    place = {}

    def yb_cp(it):
        c = it * CPG
        return pltpu.make_async_copy(
            yb.at[it], out_hbm.at[c // NC, pl.ds(c % NC, CPG), :, :, pl.ds(D, D)], s_yb)

    def put_rows(it, seg, row, n, v):
        yb[it, seg // SPC, seg % SPC, pl.ds(row, v.shape[0]), _lanes(n)] = v

    def weight_sums(src, dst):
        blocks = {}

        def get(k, j):
            blocks[k, j] = src(k, j).astype(F32)
            return blocks[k, j]

        def put(i, v):
            plain = [kj for kj, w in blocks.items() if w is v[1]]
            if i not in place:
                place[i] = (v[0], plain[0] if plain else
                            sum(isinstance(p[1], int) for p in place.values()))
            if not plain:
                dst[place[i][1]] = v[1].astype(BF16)
        return _hk_weights(get, put), len(_HK_STEPS)

    def in_sums(i):
        return [weight_sums(lambda k, j, c=c, r=r: wqkv[i * H + 8 * c + j, pl.ds(k * T + r, 16), :],
                            wsum.at[4 * i + c, :, pl.ds(r, 16), :])
                for c in range(4) for r in range(0, T, 16)]

    def xrows(s, i):
        return jnp.concatenate([xb[n, s, pl.ds(M * i, M), :].astype(F32) for n in range(NTL)], axis=1)

    def w_in(i, hd, k0, nk):
        return pltpu.bitcast(wqkv.bitcast(U32)[i * H + hd, pl.ds(k0 * T // 2, nk * T // 2), :], BF16)

    def w_out(c, n):
        return pltpu.bitcast(wo.bitcast(U32)[n, c].reshape(G * T // 2, T), BF16)

    def step(it, seg, tasks=None):
        s = 4 * it + seg
        join_in = tasks is None and seg == 0
        join_out = isinstance(seg, int) and seg == 3
        row = lax.broadcasted_iota(jnp.int32, (L, T), 0)
        col = lax.broadcasted_iota(jnp.int32, (L, T), 1)
        pos = lambda i: jnp.where(i < M, i, jnp.where(i < R, i + M, i - (R - M)))
        keep = (col < L) & ((row < M) | (pos(row) >= pos(col)))
        fill = jnp.where(col < L, -1e9, -jnp.inf).astype(F32)
        zpad = jnp.zeros((T - L, T), F32)
        tick = _Weaver((6 if join_out else 8) * H + 2 * NG, tasks or []).tick

        if tasks is not None:
            h = jnp.concatenate([mem[...]] + [xrows(s, i) for i in (1, 2, 3, 0)], axis=0)

            def proj(i, hd):
                v = _dot(h[:, :D // 2], w_in(i, hd, 0, NTL // 2))
                tick()
                v = _dot(h[:, D // 2:], w_in(i, hd, NTL // 2, NTL // 2)) + v
                tick()
                return v
        elif join_in:
            forms = _hk_forms(jnp.concatenate([mem[...]] + [xrows(s, i) for i in (1, 2, 3)], axis=0),
                              jnp.concatenate([xrows(s + i, 0) for i in range(4)], axis=0))
            lhs, done = {}, {}

            def square(i, c):
                def prod(r):
                    if r not in lhs:
                        sg, v = _sum([(t * forms[f][0], forms[f][1][:, k * T:(k + 1) * T])
                                      for (k, f), t in _HK_LHS[r].items()])
                        lhs[r] = sg, v.astype(BF16)
                    sg, at = place[r]
                    w = (pltpu.bitcast(wsum.bitcast(U32)[4 * i + c, at], BF16) if isinstance(at, int)
                         else w_in(i, 8 * c + at[1], at[0], 1))
                    return sg * lhs[r][0], _dot(lhs[r][1], w)
                acc = {}
                for st in _HK_STEPS:
                    _hk_accumulate(st, prod, acc)
                for j in range(0, 8, 2):
                    res = [_hk_result(acc, j + e) for e in range(2)]
                    for e in range(2):
                        done[i, 8 * c + j + e] = jnp.concatenate([res[e][0], res[e][1][:M]], axis=0)
                    for v in range(1, 4):
                        pre[(i * H + 8 * c + j) // 2, v - 1] = jnp.concatenate(
                            [y[M * v:M * v + M] for _, y in res], axis=0).astype(BF16)

            def proj(i, hd):
                if (i, hd) not in done:
                    square(i, hd // 8)
                return done[i, hd]
        else:
            h = jnp.concatenate([
                jnp.concatenate([mem[...], xrows(s, 1)], axis=0).astype(BF16),
                jnp.concatenate([pltpu.bitcast(xb.bitcast(U32)[n, s, pl.ds(M, M), :], BF16)
                                 for n in range(NTL)], axis=1)], axis=0)
            low = {(i, hd): _dot(h[:, :D // 2], w_in(i, hd, 0, NTL // 2))
                   for hd in range(2) for i in range(2)}

            def proj(i, hd):
                v = (_dot(h[:, D // 2:], w_in(i, hd, NTL // 2, NTL // 2)) + low[i, hd]
                     if (i, hd) in low else _dot(h, w_in(i, hd, 0, NTL)))
                first = pre[(i * H + hd) // 2, seg - 1].astype(F32)[M * (hd % 2):M * (hd % 2) + M]
                return jnp.concatenate([v, first], axis=0)

        def pad(v):
            return jnp.concatenate([v, zpad], axis=0).astype(BF16)

        lags = (0, 2, 2, 4, 5) if join_in else (0, 1, 1, 2, 5 if join_out else 3)
        qkv, es, att, oforms, acc = {}, {}, {}, {}, {}
        todo = list(_HK_STEPS)
        for op, g in ((op, g - lag) for g in range(NG + lags[-1])
                      for op, lag in zip(("qk", "s", "v", "p", "o"), lags) if 0 <= g - lag < NG):
            heads = range(g * G, g * G + G)
            if op == "s":
                for hd in heads:
                    sc = jnp.where(keep, _dot(qkv["q", hd], pad(qkv["k", hd]), NT) * scale, fill)
                    e = jnp.exp(sc - jnp.max(sc, axis=1, keepdims=True))
                    es[hd] = e, pltpu.reciprocal(jnp.sum(e, axis=1, keepdims=True), full_range=False)
                tick()
            elif op == "p":
                for hd in heads:
                    o = _dot(es[hd][0], pad(qkv["v", hd])) * es[hd][1]
                    if join_out:
                        att[hd] = o
                    else:
                        att[hd] = o[:R].astype(BF16)
                        opre[seg, :, _lanes(hd)] = o[R:]
                tick()
            elif op != "o":
                for hd in heads:
                    for x in op:
                        qkv[x, hd] = proj("qkv".index(x), hd)
            elif join_out:
                o = jnp.concatenate([att[hd] for hd in heads], axis=1)
                late = opre[:, :, pl.ds(g * G * T, G * T)].reshape(3 * M, G * T)
                oforms[g] = _hk_forms(o[:R], jnp.concatenate([o[R:], late], axis=0))

                def prod(r):
                    sg, v = _sum([(t * oforms[k][f][0], oforms[k][f][1])
                                  for (k, f), t in _HK_LHS[r].items()])
                    at = place[r][1]
                    w = (pltpu.bitcast(wosum.bitcast(U32)[at].reshape(G * T // 2, T), BF16)
                         if isinstance(at, int) else w_out(*at))
                    return sg * place[r][0], _dot(v.astype(BF16), w)
                for _ in range(g + 1):
                    _hk_accumulate(todo.pop(0), prod, acc)
            else:
                o = jnp.concatenate([att[hd] for hd in heads], axis=1)
                for n in range(NTL):
                    part = _dot(o, w_out(g, n))
                    acc[n] = part + acc[n] if g else part
                    tick()
        for n in range(NTL):
            if join_out:
                out, late = _hk_result(acc, n)
                for v in range(4):
                    put_rows(it, (v + 3) % 4, 0, n, late[M * v:M * v + M])
            else:
                out = acc[n]
            mem[:, _lanes(n)] = out[:M]
            put_rows(it, seg, M, n, out[M:])

    def first_steps(i, _):
        step(0, i, in_sums(i)[:24] + [
            weight_sums(lambda k, j, r=r: wo[j, k, 10 * i + r], wosum.at[:, 10 * i + r])
            for r in range(12)])

    def four_steps(it, _):
        for seg in range(4):
            step(it, seg)
        yb_cp(it).start()

    mem[...] = mem0[...].astype(F32)
    lax.fori_loop(0, 3, first_steps, None)
    step(0, 3, _join(in_sums(i)[24:] for i in range(3)))
    fence()
    _start(ya_cp + [yb_cp(0)])
    lax.fori_loop(1, NSEG // 4, four_steps, None)
    _wait([yb_cp(it) for it in range(NSEG // 4)])


def _kernel(xa_hbm, lre_hbm, lim_hbm, bre_hbm, bim_hbm, cre_hbm, cim_hbm, ldt_hbm, dsk_hbm,
            xb_hbm, mem0_hbm, wq_hbm, wk_hbm, wv_hbm, wo_hbm, out_hbm,
            ya, xb, mem0, wqkv, wo, s_w, s_late, s_ya, s_fence):
    NTL, NSEG, SEG, _ = xb.shape
    SPC, D = ya.shape[1], ya.shape[-1]
    TB = SPC * SEG
    H = wqkv.shape[0] // 3
    M = mem0.shape[0]

    def fence():
        pl.semaphore_signal(s_fence)
        pl.semaphore_wait(s_fence)

    w_cp = [[pltpu.make_async_copy(w.bitcast(U32).at[:, (hd % 2) * (H // 2) + hd // 2, :],
                                   wqkv.bitcast(U32).at[i * H + hd], s_w.at[(i * H + hd) // 8])
             for hd in range(c, c + 8)]
            for i, w in enumerate((wq_hbm, wk_hbm, wv_hbm)) for c in range(0, H, 8)]
    late_cp = [[pltpu.make_async_copy(src.at[..., _lanes(n)], dst.at[n], s_late)
                for n in range(c, c + 2) for src, dst in ((wo_hbm, wo), (xb_hbm, xb))]
               for c in range(0, NTL, 2)]
    late_cp[0].append(pltpu.make_async_copy(mem0_hbm, mem0, s_late))

    ya_cp = [pltpu.make_async_copy(ya.at[:, :, :, c, :], out_hbm.at[:, c, :, :, pl.ds(0, D)], s_ya)
             for c in range(NC)]

    pl.run_scoped(
        functools.partial(_s5, xa_hbm, (lre_hbm, lim_hbm, ldt_hbm, dsk_hbm), (bre_hbm, bim_hbm),
                          (cre_hbm, cim_hbm), ya, wqkv, w_cp, late_cp, fence),
        pltpu.VMEM((4, NTL, T), BF16),
        pltpu.VMEM((NB, TB // 2, NC, D), U32),
        pltpu.VMEM((2, D, D), BF16),
        pltpu.VMEM((2, D, D), BF16),
        pltpu.VMEM((NB, NTL, TB, 2 * NC, T), BF16),
        pltpu.VMEM((17 + 2 * NB, NC, D), F32),
        *[pltpu.VMEM((4, 49, T, T), BF16)] * 5,
        *[pltpu.VMEM((49, T, T), F32)] * 4,
        pltpu.SemaphoreType.DMA,
        pltpu.SemaphoreType.DMA((NB + 1,)),
        pltpu.SemaphoreType.DMA((8,)),
        pltpu.SemaphoreType.DMA((2,)),
    )
    _wait(_join(late_cp))
    pl.run_scoped(
        functools.partial(_transformer, mem0, out_hbm, wqkv, wo, xb, ya_cp, fence),
        pltpu.VMEM((3 * H // 8, _HK_SUMS, T, T), BF16),
        pltpu.VMEM((_HK_SUMS, *wo.shape[2:]), BF16),
        pltpu.VMEM((3 * H // 2, 3, 2 * M, T), BF16),
        pltpu.VMEM((3, M, H * T), F32),
        pltpu.VMEM((NSEG // 4, 4 // SPC, SPC, SEG, D), F32),
        pltpu.VMEM((M, D), F32),
        pltpu.SemaphoreType.DMA,
    )
    _wait(ya_cp)


@functools.partial(jax.jit, static_argnames=("B_seg_len",))
def pallas_concat_heads__ssm_conv_s5__memory_aug_recurrent_mem_tr__prompt_kernel(
    A_x, A_Lambda_re, A_Lambda_im, A_B_re, A_B_im, A_C_re, A_C_im, A_log_dt, A_Dskip,
    B_x, B_mem0, B_Wq, B_Wk, B_Wv, B_Wo, B_seg_len,
):
    _, S, D = A_x.shape
    _, H, Dh = B_Wq.shape
    M = B_mem0.shape[1]
    SEG = int(B_seg_len)
    TB = S // (NB * NC)
    assert (S, D, H, Dh, M, SEG) == (2048, 1024, 32, 128, 8, 32)
    hbm = pl.BlockSpec(memory_space=pl.ANY)
    tile = lambda v: v.reshape(D // T, T)
    pairs = lambda w: w.reshape(D // 2, 2 * H, Dh)
    out = pl.pallas_call(
        _kernel,
        out_shape=jax.ShapeDtypeStruct((NB, NC, TB // SEG, SEG, 2 * D), F32),
        in_specs=[hbm] * 15,
        out_specs=hbm,
        scratch_shapes=[
            pltpu.VMEM((NB, TB // SEG, SEG, NC, D), F32),
            pltpu.VMEM((D // T, S // SEG, SEG, T), BF16),
            pltpu.VMEM((M, D), BF16),
            pltpu.VMEM((3 * H, D, T), BF16),
            pltpu.VMEM((D // T, 8, H * Dh // T, 16, T), BF16),
            pltpu.SemaphoreType.DMA((3 * H // 8,)),
            pltpu.SemaphoreType.DMA,
            pltpu.SemaphoreType.DMA,
            pltpu.SemaphoreType.REGULAR,
        ],
        compiler_params=pltpu.CompilerParams(vmem_limit_bytes=116 * 1024 * 1024),
    )(A_x.reshape(NB, NC, TB, D), tile(A_Lambda_re), tile(A_Lambda_im),
      A_B_re, A_B_im, A_C_re, A_C_im, tile(A_log_dt), tile(A_Dskip),
      B_x.reshape(S // SEG, SEG, D), B_mem0.reshape(M, D),
      pairs(B_Wq), pairs(B_Wk), pairs(B_Wv), B_Wo.reshape(8, H * Dh // T, 16, D))
    return out.reshape(1, S, 2 * D)
```
